```python
import jax
import jax.numpy as jnp

def _softmax(x, axis=-1):
    return jax.nn.softmax(x, axis=axis)
def _gelu(x):
    return jax.nn.gelu(x, approximate=True)
def _silu(x):
    return jax.nn.silu(x)
def _sigmoid(x):
    return jax.nn.sigmoid(x)
def _layernorm(x, axis=-1, eps=1e-5):
    m = jnp.mean(x, axis=axis, keepdims=True)
    v = jnp.var(x, axis=axis, keepdims=True)
    return (x - m) / jnp.sqrt(v + eps)
def _scatter_add(tgt, idx, src, axis=0):
    return tgt.at[idx].add(src)
def _segment_sum(src, seg, n):
    return jax.ops.segment_sum(src, seg, n)
class _Rng:
    def __init__(self, key):
        self._k = key
    def _next(self):
        self._k, sub = jax.random.split(self._k)
        return sub
    def normal(self, shape):
        return jax.random.normal(self._next(), shape, dtype=jnp.bfloat16)
    def randint(self, lo, hi, shape):
        return jax.random.randint(self._next(), shape, lo, hi, dtype=jnp.int32)
    def uniform(self, shape, lo=0.0, hi=1.0):
        return jax.random.uniform(self._next(), shape, jnp.bfloat16, lo, hi)
    def permutation(self, n):
        return jax.random.permutation(self._next(), n)


kernel_name = 'standalone__groupnorm__prompt'

def setup_inputs():
    _rng = _Rng(jax.random.key(int.from_bytes(__import__("os").urandom(4), "little")))
    _w = (lambda a: (lambda t: t.astype(jnp.bfloat16) if jnp.issubdtype(t.dtype, jnp.floating) else t)(jnp.asarray(a)))
    B = 2
    G = 32
    cpg = max(1, 1024 // G)
    C = G * cpg
    H, W = 32, 2048
    return {
        "x": _w((lambda *s: _rng.normal(s) * 0.05)(B, C, H, W)),
        "g": _w((lambda *s: _rng.normal(s) * 0.05)(C) + 1.0),
        "b": _w((lambda *s: _rng.normal(s) * 0.05)(C)),
    }

def reference(x, g, b):
    G = 32
    B, C, H, W = x.shape[0], x.shape[1], x.shape[2], x.shape[3]
    xr = x.reshape(B, G, C // G, H, W)
    mu = xr.mean(axis=(2, 3, 4), keepdims=True)
    var = ((xr - mu) ** 2).mean(axis=(2, 3, 4), keepdims=True)
    xn = (xr - mu) / jnp.sqrt(var + 1e-5)
    xn = xn.reshape(B, C, H, W)
    return xn * g[None, :, None, None] + b[None, :, None, None]
```

```python
import jax
import jax.numpy as jnp
from jax import lax
import jax.experimental.pallas as pl
import jax.experimental.pallas.tpu as pltpu

_GROUPS = 32
_EPS = 1e-5


@jax.jit
def pallas_standalone__groupnorm__prompt_kernel(x: jax.Array, g: jax.Array, b: jax.Array):
    B, C, H, W = x.shape
    cpg = C // _GROUPS
    inv_n = 1.0 / (cpg * H * W)

    def kernel(g_ref, b_ref, x_ref, o_ref):
        grp = pl.program_id(1)

        def sum_body(c, acc):
            return acc + x_ref[0, c].astype(jnp.float32)

        s = lax.fori_loop(0, cpg, sum_body, jnp.zeros((H, W), jnp.float32))
        mu = jnp.sum(s, keepdims=True) * inv_n

        def var_body(c, acc):
            d = x_ref[0, c].astype(jnp.float32) - mu
            return acc + d * d

        v = lax.fori_loop(0, cpg, var_body, jnp.zeros((H, W), jnp.float32))
        rstd = lax.rsqrt(jnp.sum(v, keepdims=True) * inv_n + _EPS)

        def out_body(c, carry):
            d = x_ref[0, c].astype(jnp.float32) - mu
            o_ref[0, c] = (d * (rstd * g_ref[grp * cpg + c]) + b_ref[grp * cpg + c]).astype(o_ref.dtype)
            return carry

        lax.fori_loop(0, cpg, out_body, 0)

    return pl.pallas_call(
        kernel,
        grid=(B, _GROUPS),
        in_specs=[
            pl.BlockSpec(memory_space=pltpu.SMEM),
            pl.BlockSpec(memory_space=pltpu.SMEM),
            pl.BlockSpec((1, cpg, H, W), lambda i, j: (i, j, 0, 0)),
        ],
        out_specs=pl.BlockSpec((1, cpg, H, W), lambda i, j: (i, j, 0, 0)),
        out_shape=jax.ShapeDtypeStruct(x.shape, x.dtype),
        compiler_params=pltpu.CompilerParams(
            dimension_semantics=("arbitrary", "arbitrary"), vmem_limit_bytes=64 << 20
        ),
    )(g.astype(jnp.float32), b.astype(jnp.float32), x)
```

```python
import jax
import jax.numpy as jnp
from jax import lax
import jax.experimental.pallas as pl
import jax.experimental.pallas.tpu as pltpu

GROUPS = 32
EPS = 1e-5
LANES = 128


def build(lag=3, units=8, rtail=8, wtail=2, rsplit=(2, 3, 3), wsplit=(8, 12, 12), sub=128, nacc=4,
          compute=True, dma=True, nobounds=True, rorder=None):
    def f(x, g, b):
        B, C, H, W = x.shape
        cpg = C // GROUPS
        ch_rows = H * W // LANES
        n_units = B * GROUPS // 2
        n_phase = n_units // units
        half = 4 * ch_rows
        inv_n = 1.0 / (cpg * H * W)
        RD, WR = 128, 64
        n_rd, n_wr = half // RD, half // WR
        order = rorder or [int(f"{u:04b}"[::-1], 2) for u in range(16)]
        steps = 4 * units

        def kernel(x_hbm, g_hbm, b_hbm, o_hbm, buf, g_v, b_v, g_tab, b_tab, rsem, wsem, psem):
            ph, s = pl.program_id(0), pl.program_id(1)

            def wait(ref, sem):
                if dma:
                    pltpu.make_async_copy(ref, ref, sem).wait()

            def issue_reads(j0, nj):
                slot = s >> 1
                def body(jj, carry):
                    j = (s & 1) * (n_rd // 2) + jj
                    r0 = pl.multiple_of(j * RD, RD)
                    last = jnp.logical_and(slot == units - 1, j == n_rd - 1)
                    tail_sem = jnp.where(last, units, slot)
                    for u, r in enumerate(order):
                        sem = rsem.at[tail_sem] if u >= 16 - rtail else rsem.at[slot]
                        pltpu.make_async_copy(x_hbm.at[ph * units + slot, r // 2, r % 2, pl.ds(r0, RD)],
                                              buf.at[slot, r // 2, r % 2, pl.ds(r0, RD)], sem).start(priority=u % 2)
                    return carry
                lax.fori_loop(j0, j0 + nj, body, 0)

            def issue_writes(j0, nj):
                slot = (s >> 1) - units
                def body(j, carry):
                    r0 = pl.multiple_of(j * WR, WR)
                    is_tail = jnp.logical_and(s == steps - 1, j >= n_wr - wtail)
                    pltpu.make_async_copy(buf.at[slot, :, s & 1, pl.ds(r0, WR)],
                                          o_hbm.at[ph * units + slot, :, s & 1, pl.ds(r0, WR)],
                                          wsem.at[is_tail.astype(jnp.int32)]).start()
                    return carry
                lax.fori_loop(j0, j0 + nj, body, 0)

            def issue(part):
                if not dma:
                    return
                if rsplit[part]:
                    @pl.when(s < 2 * units)
                    def _():
                        issue_reads(sum(rsplit[:part]), rsplit[part])
                if wsplit[part]:
                    @pl.when(s >= 2 * units)
                    def _():
                        issue_writes(sum(wsplit[:part]), wsplit[part])

            def wait_read_head():
                wait(buf.at[units - 1, :, :, pl.ds(0, half - RD)], rsem.at[units - 1])
                for u, r in enumerate(order[:16 - rtail]):
                    wait(buf.at[units - 1, r // 2, r % 2, pl.ds(half - RD, RD)], rsem.at[units - 1])

            def wait_read_tail():
                for u, r in enumerate(order[16 - rtail:]):
                    wait(buf.at[units - 1, r // 2, r % 2, pl.ds(half - RD, RD)], rsem.at[units])

            def wait_write_head():
                wait(buf.at[pl.ds(0, units - 1)], wsem.at[0])
                wait(buf.at[units - 1, :, 0], wsem.at[0])
                wait(buf.at[units - 1, :, 1, pl.ds(0, half - wtail * WR)], wsem.at[0])

            def wait_write_tail():
                if wtail:
                    wait(buf.at[units - 1, :, 1, pl.ds(half - wtail * WR, wtail * WR)], wsem.at[1])

            c = s - lag
            active = jnp.logical_and(c >= 0, c < 2 * units)
            trips = jnp.where(active, 8, 0) if compute else 0

            def piece(i, k):
                return (c >> 1, (c & 1) * 4 + (i >> 1), i & 1, pl.ds(k * sub, sub))

            def fold(v):
                return v.reshape(sub // (8 * nacc), 8 * nacc, LANES).sum(axis=0)

            @pl.when(jnp.logical_and(s == 0, ph > 0))
            def _():
                wait_write_head()
            @pl.when(jnp.logical_and(s == 1, ph > 0))
            def _():
                wait_write_tail()
            @pl.when(s == 2 * units)
            def _():
                wait_read_head()

            issue(0)

            @pl.when(jnp.logical_and(ph == 0, s == 0))
            def _():
                pltpu.make_async_copy(g_hbm, g_v, psem.at[0]).start()
                pltpu.make_async_copy(b_hbm, b_v, psem.at[1]).start()
            @pl.when(jnp.logical_and(ph == 0, s == 1))
            def _():
                pltpu.make_async_copy(g_hbm, g_v, psem.at[0]).wait()
                pltpu.make_async_copy(b_hbm, b_v, psem.at[1]).wait()
                for src, dst in ((g_v, g_tab), (b_v, b_tab)):
                    v = src[...].astype(jnp.float32).reshape(1, C)
                    for k in range(C // LANES):
                        dst[pl.ds(k * LANES, LANES), :] = jnp.broadcast_to(v[:, k * LANES:(k + 1) * LANES], (LANES, LANES)).T

            @pl.when(jnp.logical_and(active, (c & 1) == 0))
            def _():
                @pl.when(c < 2 * units - 2)
                def _():
                    wait(buf.at[c >> 1], rsem.at[c >> 1])
                @pl.when(c == 2 * units - 2)
                def _():
                    wait_read_tail()

            def p1(i, acc):
                for k in range(half // sub):
                    acc = acc + fold(buf[piece(i, k)].astype(jnp.float32))
                return acc
            acc = lax.fori_loop(0, trips, p1, jnp.zeros((8 * nacc, LANES), jnp.float32))
            mu = jnp.sum(acc, keepdims=True) * inv_n

            issue(1)

            def p2(i, acc):
                for k in range(half // sub):
                    d = buf[piece(i, k)].astype(jnp.float32) - mu
                    acc = acc + fold(d * d)
                return acc
            acc = lax.fori_loop(0, trips, p2, jnp.zeros((8 * nacc, LANES), jnp.float32))
            rstd = 1.0 / jnp.sqrt(jnp.sum(acc, keepdims=True) * inv_n + EPS)

            issue(2)

            def p3(i, carry):
                ch0 = ((ph * 2 * units + c) & (GROUPS - 1)) * cpg + i * 4
                for q in range(4):
                    scale = g_tab[pl.ds(ch0 + q, 1), :] * rstd
                    shift = b_tab[pl.ds(ch0 + q, 1), :]
                    for k in range(q * ch_rows // sub, (q + 1) * ch_rows // sub):
                        d = buf[piece(i, k)].astype(jnp.float32) - mu
                        buf[piece(i, k)] = (d * scale + shift).astype(buf.dtype)
                return carry
            lax.fori_loop(0, trips, p3, 0)

            @pl.when(jnp.logical_and(ph == n_phase - 1, s == steps - 1))
            def _():
                wait_write_head()
                wait_write_tail()

        xt = x.reshape(B * C * H // 8, 8, W // LANES, LANES).transpose(0, 2, 1, 3).reshape(n_units, 8, 2, half, LANES)
        out = pl.pallas_call(
            kernel,
            grid=(n_phase, steps),
            in_specs=[pl.BlockSpec(memory_space=pl.ANY)] * 3,
            out_specs=pl.BlockSpec(memory_space=pl.ANY),
            out_shape=jax.ShapeDtypeStruct(xt.shape, x.dtype),
            scratch_shapes=[
                pltpu.VMEM((units, 8, 2, half, LANES), x.dtype),
                pltpu.VMEM((C,), g.dtype), pltpu.VMEM((C,), b.dtype),
                pltpu.VMEM((C, LANES), jnp.float32), pltpu.VMEM((C, LANES), jnp.float32),
                pltpu.SemaphoreType.DMA((units + 1,)), pltpu.SemaphoreType.DMA((2,)), pltpu.SemaphoreType.DMA((2,)),
            ],
            compiler_params=pltpu.CompilerParams(vmem_limit_bytes=100 << 20, disable_bounds_checks=nobounds,
                                                 dimension_semantics=("arbitrary", "arbitrary")),
        )(xt, g, b)
        return out.reshape(B * C * H // 8, W // LANES, 8, LANES).transpose(0, 2, 1, 3).reshape(x.shape)
    return f


_impl = build(lag=12, nobounds=False)


@jax.jit
def pallas_standalone__groupnorm__prompt_kernel(x: jax.Array, g: jax.Array, b: jax.Array):
    return _impl(x, g, b)
```

```python
import jax
import jax.numpy as jnp
from jax import lax
import jax.experimental.pallas as pl
import jax.experimental.pallas.tpu as pltpu

GROUPS = 32
EPS = 1e-5
LANES = 128


def build(ahead=2, U=4, rtail=4, wtail=2, rsplit=(4, 6, 6), wsplit=(8, 12, 12), sub_r=8, sub_c=2048, acc_c=512,
          compute=True, nobounds=True, order=(0, 4, 1, 5, 2, 6, 3, 7)):
    def f(x, g, b):
        B, C, H, W = x.shape
        cpg = C // GROUPS
        n_units = B * GROUPS // 4
        n_phase = n_units // U
        cpr = cpg // 4
        reg = cpr * H
        inv_n = 1.0 / (cpg * H * W)
        PR, PC = 8, W // 2
        n_p = reg // PR
        lag = 4 * U - ahead

        def kernel(x_hbm, g_hbm, b_hbm, o_hbm, buf, g_v, b_v, g_tab, b_tab, rsem, wsem, psem):
            def rd(ph, slot, idx, sem):
                return pltpu.make_async_copy(x_hbm.at[(ph * U + slot, *idx)], buf.at[(slot, *idx)], rsem.at[sem])

            def wr(ph, slot, idx, sem):
                return pltpu.make_async_copy(buf.at[(slot, *idx)], o_hbm.at[(ph * U + slot, *idx)], wsem.at[sem])

            def band(j):
                return pl.ds(pl.multiple_of(j * PR, PR), PR)

            r_head, w_head = (n_p - rtail // 2) * PR, (n_p - wtail // 2) * PR

            def wait_write_head(ph):
                for k in range(2 * U - 1):
                    wr(ph, k // 2, (pl.ds(8 * (k % 2), 8),), k).wait()
                wr(ph, U - 1, (pl.ds(8, 8), pl.ds(0, w_head)), 2 * U - 1).wait()

            def wait_write_tail(ph):
                wr(ph, U - 1, (pl.ds(8, 8), pl.ds(w_head, reg - w_head)), 2 * U).wait()

            def step(ph, s):
                def issue(part):
                    @pl.when(s < 4 * U)
                    def _():
                        slot = s >> 2
                        def body(jj, carry):
                            j = (s & 3) * (n_p // 4) + jj
                            sem = jnp.where(jnp.logical_and(slot == U - 1, j * PR >= r_head), U, slot)
                            for w in range(2):
                                for u, a in enumerate(order):
                                    rd(ph, slot, (pl.ds(2 * a, 2), band(j), pl.ds(w * PC, PC)), sem).start(priority=u % 2)
                            return carry
                        lax.fori_loop(sum(rsplit[:part]) // 2, sum(rsplit[:part + 1]) // 2, body, 0)

                    @pl.when(s >= 4 * U)
                    def _():
                        k = (s >> 1) - 2 * U
                        def body(jj, carry):
                            j = (s & 1) * (n_p // 2) + jj
                            sem = jnp.where(jnp.logical_and(k == 2 * U - 1, j * PR >= w_head), 2 * U, k)
                            for w in range(2):
                                wr(ph, k >> 1, (pl.ds(8 * (k & 1), 8), band(j), pl.ds(w * PC, PC)), sem).start()
                            return carry
                        lax.fori_loop(sum(wsplit[:part]) // 2, sum(wsplit[:part + 1]) // 2, body, 0)

                c = s - lag
                active = jnp.logical_and(c >= 0, c < 4 * U)
                trips = jnp.where(active, 8, 0) if compute else 0
                half = reg // 2

                def slab(i):
                    return buf.at[c >> 2, (c & 3) * 4 + (i >> 1), pl.ds(pl.multiple_of((i & 1) * half, half), half)]

                def pieces(i, r_lo, r_hi):
                    for r in range(r_lo, r_hi, sub_r):
                        for w in range(0, W, sub_c):
                            yield (pl.ds(r, sub_r), pl.ds(w, sub_c))

                def fold(acc, v):
                    for w in range(0, sub_c, acc_c):
                        acc = acc + v[:, w:w + acc_c]
                    return acc

                @pl.when(jnp.logical_and(s == 0, ph > 0))
                def _():
                    wait_write_head(ph - 1)
                @pl.when(jnp.logical_and(s == 1, ph > 0))
                def _():
                    wait_write_tail(ph - 1)
                @pl.when(s == 4 * U)
                def _():
                    rd(ph, U - 1, (slice(None), pl.ds(0, r_head)), U - 1).wait()

                issue(0)

                @pl.when(jnp.logical_and(ph == 0, s == 0))
                def _():
                    pltpu.make_async_copy(g_hbm, g_v, psem.at[0]).start()
                    pltpu.make_async_copy(b_hbm, b_v, psem.at[1]).start()
                @pl.when(jnp.logical_and(ph == 0, s == 1))
                def _():
                    pltpu.make_async_copy(g_hbm, g_v, psem.at[0]).wait()
                    pltpu.make_async_copy(b_hbm, b_v, psem.at[1]).wait()
                    for src, dst in ((g_v, g_tab), (b_v, b_tab)):
                        v = src[...].astype(jnp.float32).reshape(1, C)
                        for k in range(C // LANES):
                            dst[pl.ds(k * LANES, LANES), :] = jnp.broadcast_to(v[:, k * LANES:(k + 1) * LANES], (LANES, LANES)).T

                @pl.when(jnp.logical_and(active, (c & 3) == 0))
                def _():
                    @pl.when(c < 4 * U - 4)
                    def _():
                        rd(ph, c >> 2, (), c >> 2).wait()
                    @pl.when(c == 4 * U - 4)
                    def _():
                        rd(ph, U - 1, (slice(None), pl.ds(r_head, reg - r_head)), U).wait()

                def p1(i, acc):
                    v = slab(i)
                    for p in pieces(i, 0, half):
                        acc = fold(acc, v[p].astype(jnp.float32))
                    return acc
                acc = lax.fori_loop(0, trips, p1, jnp.zeros((sub_r, acc_c), jnp.float32))
                mu = jnp.sum(acc, keepdims=True) * inv_n

                issue(1)

                def p2(i, acc):
                    v = slab(i)
                    for p in pieces(i, 0, half):
                        d = v[p].astype(jnp.float32) - mu
                        acc = fold(acc, d * d)
                    return acc
                acc = lax.fori_loop(0, trips, p2, jnp.zeros((sub_r, acc_c), jnp.float32))
                rstd = 1.0 / jnp.sqrt(jnp.sum(acc, keepdims=True) * inv_n + EPS)

                issue(2)

                def p3(i, carry):
                    v = slab(i)
                    ch0 = ((ph * U * 4 + c) & (GROUPS - 1)) * cpg + i * (cpr // 2)
                    for q in range(cpr // 2):
                        scale = jnp.tile(g_tab[pl.ds(ch0 + q, 1), :] * rstd, (1, sub_c // LANES))
                        shift = jnp.tile(b_tab[pl.ds(ch0 + q, 1), :], (1, sub_c // LANES))
                        for p in pieces(i, q * H, (q + 1) * H):
                            d = v[p].astype(jnp.float32) - mu
                            v[p] = (d * scale + shift).astype(buf.dtype)
                    return carry
                lax.fori_loop(0, trips, p3, 0)

            @pl.loop(0, n_phase)
            def _(ph):
                @pl.loop(0, 8 * U)
                def _(s):
                    step(ph, s)

            wait_write_head(n_phase - 1)
            wait_write_tail(n_phase - 1)

        xt = x.reshape(n_units, 16, reg, W)
        out = pl.pallas_call(
            kernel,
            in_specs=[pl.BlockSpec(memory_space=pl.ANY)] * 3,
            out_specs=pl.BlockSpec(memory_space=pl.ANY),
            out_shape=jax.ShapeDtypeStruct(xt.shape, x.dtype),
            scratch_shapes=[
                pltpu.VMEM((U, 16, reg, W), x.dtype),
                pltpu.VMEM((C,), g.dtype), pltpu.VMEM((C,), b.dtype),
                pltpu.VMEM((C, LANES), jnp.float32), pltpu.VMEM((C, LANES), jnp.float32),
                pltpu.SemaphoreType.DMA((U + 1,)), pltpu.SemaphoreType.DMA((2 * U + 1,)), pltpu.SemaphoreType.DMA((2,)),
            ],
            compiler_params=pltpu.CompilerParams(vmem_limit_bytes=(U * 16 + 6) << 20, disable_bounds_checks=nobounds),
        )(xt, g, b)
        return out.reshape(x.shape)
    return f


_impl = build(nobounds=False)


@jax.jit
def pallas_standalone__groupnorm__prompt_kernel(x: jax.Array, g: jax.Array, b: jax.Array):
    return _impl(x, g, b)
```

```python
import jax
import jax.numpy as jnp
from jax import lax
import jax.experimental.pallas as pl
import jax.experimental.pallas.tpu as pltpu

_GROUPS = 32
_EPS = 1e-5
_LANES = 128

_PHASES = 3
_BAND = 8
_PAIR_ORDER = (0, 4, 1, 5, 2, 6, 3, 7)
_READ_TAIL = 2
_WRITE_TAIL = 1
_AHEAD = 2
_ACC_LANES = 4 * _LANES


@jax.jit
def pallas_standalone__groupnorm__prompt_kernel(x: jax.Array, g: jax.Array, b: jax.Array):
    B, C, H, W = x.shape
    cpg = C // _GROUPS
    units = B * _GROUPS // 4
    slots = pl.cdiv(units, _PHASES)
    short_phases = slots * _PHASES - units
    rows = cpg * H // 4
    bands = rows // _BAND
    slab_ch, slab_rows = cpg // 8, rows // 2
    read_head, write_head = (bands - _READ_TAIL) * _BAND, (bands - _WRITE_TAIL) * _BAND
    inv_n = 1.0 / (cpg * H * W)
    assert C % _LANES == 0 and cpg % 8 == 0 and H % _BAND == 0 and W % _ACC_LANES == 0
    assert bands % 32 == 0 and slots >= 3

    def kernel(x_hbm, g_hbm, b_hbm, o_hbm, buf, g_vmem, b_vmem, g_tab, b_tab, rsem, wsem, psem):
        def read(base, slot, idx, sem):
            src, dst = x_hbm.at[(base + slot, *idx)], buf.at[(slot, *idx)]
            return pltpu.make_async_copy(src, dst, rsem.at[sem])

        def write(base, pair, idx, sem):
            idx = (pl.ds(8 * (pair & 1), 8), *idx)
            src, dst = buf.at[(pair >> 1, *idx)], o_hbm.at[(base + (pair >> 1), *idx)]
            return pltpu.make_async_copy(src, dst, wsem.at[sem])

        def piece(band, side):
            return pl.ds(pl.multiple_of(band * _BAND, _BAND), _BAND), pl.ds(side * W // 2, W // 2)

        def wait_write_tail(base):
            write(base, 2 * slots - 1, (pl.ds(write_head, rows - write_head),), 2 * slots).wait()

        param_copies = (
            pltpu.make_async_copy(g_hbm, g_vmem, psem.at[0]),
            pltpu.make_async_copy(b_hbm, b_vmem, psem.at[1]),
        )

        def step(phase, base, first, t):
            n = 4 * (slots - first)
            reading = t < n
            s = jnp.where(reading, t, t - n) + 4 * first
            slot, pair = s >> 2, s >> 1
            grp = t - (n - _AHEAD) + 4 * first

            def start_copies(lo, hi):
                @pl.when(reading)
                def _():
                    @pl.loop(lo * bands // 32, hi * bands // 32)
                    def _(i):
                        band = (s & 3) * (bands // 4) + i
                        tail = jnp.logical_and(slot == slots - 1, band >= bands - _READ_TAIL)
                        sem = jnp.where(tail, slots, slot)
                        for side in range(2):
                            for k, r in enumerate(_PAIR_ORDER):
                                idx = (pl.ds(2 * r, 2), *piece(band, side))
                                read(base, slot, idx, sem).start(priority=k % 2)

                @pl.when(jnp.logical_not(reading))
                def _():
                    @pl.loop(lo * bands // 16, hi * bands // 16)
                    def _(i):
                        band = (s & 1) * (bands // 2) + i
                        tail = jnp.logical_and(pair == 2 * slots - 1, band >= bands - _WRITE_TAIL)
                        sem = jnp.where(tail, 2 * slots, pair)
                        for side in range(2):
                            write(base, pair, piece(band, side), sem).start()

            @pl.when(jnp.logical_and(t == 1, phase > 0))
            def _():
                wait_write_tail(base + first - slots)

            @pl.when(jnp.logical_and(reading, jnp.logical_and((s & 3) == 1, slot > first)))
            def _():
                read(base, slot - 1, (), slot - 1).wait()

            @pl.when(t == n)
            def _():
                read(base, slots - 1, (slice(None), pl.ds(0, read_head)), slots - 1).wait()

            @pl.when(t == n + 1)
            def _():
                read(base, slots - 1, (slice(None), pl.ds(read_head, rows - read_head)), slots).wait()

            @pl.when(jnp.logical_and(t >= n + 4, (s & 1) == 1))
            def _():
                write(base, pair - 2, (), pair - 2).wait()

            start_copies(0, 2)

            @pl.when(jnp.logical_and(phase == 0, t == 0))
            def _():
                for copy in param_copies:
                    copy.start()

            @pl.when(jnp.logical_and(phase == 0, t == 1))
            def _():
                for copy in param_copies:
                    copy.wait()
                for src, tab in ((g_vmem, g_tab), (b_vmem, b_tab)):
                    v = src[...].astype(jnp.float32).reshape(1, C)
                    for k in range(0, C, _LANES):
                        tab[pl.ds(k, _LANES), :] = jnp.broadcast_to(v[:, k : k + _LANES], (_LANES, _LANES)).T

            num_slabs = jnp.where(jnp.logical_and(grp >= 4 * first, grp < 4 * slots), 8, 0)

            def slab(i):
                row0 = pl.multiple_of((i & 1) * slab_rows, slab_rows)
                return buf.at[grp >> 2, (grp & 3) * 4 + (i >> 1), pl.ds(row0, slab_rows)]

            def mean_of(fn):
                def body(i, acc):
                    ref = slab(i)
                    for r in range(0, slab_rows, _BAND):
                        v = fn(ref[pl.ds(r, _BAND), :].astype(jnp.float32))
                        for w in range(0, W, _ACC_LANES):
                            acc = acc + v[:, w : w + _ACC_LANES]
                    return acc

                acc = lax.fori_loop(0, num_slabs, body, jnp.zeros((_BAND, _ACC_LANES), jnp.float32))
                return jnp.sum(acc, keepdims=True) * inv_n

            mu = mean_of(lambda v: v)
            start_copies(2, 5)
            var = mean_of(lambda v: jnp.square(v - mu))
            rstd = 1.0 / jnp.sqrt(var + _EPS)
            start_copies(5, 8)

            @pl.loop(0, num_slabs)
            def _(i):
                ref = slab(i)
                ch0 = ((4 * base + grp) & (_GROUPS - 1)) * cpg + i * slab_ch
                for c in range(slab_ch):
                    scale = jnp.tile(g_tab[pl.ds(ch0 + c, 1), :] * rstd, (1, W // _LANES))
                    shift = jnp.tile(b_tab[pl.ds(ch0 + c, 1), :], (1, W // _LANES))
                    for r in range(c * H, (c + 1) * H, _BAND):
                        v = ref[pl.ds(r, _BAND), :].astype(jnp.float32)
                        ref[pl.ds(r, _BAND), :] = ((v - mu) * scale + shift).astype(ref.dtype)

        @pl.loop(0, _PHASES)
        def _(phase):
            first = jnp.where(phase < short_phases, 1, 0)
            base = phase * slots - jnp.minimum(phase + 1, short_phases)

            @pl.loop(0, 8 * (slots - first))
            def _(t):
                step(phase, base, first, t)

            write(base, 2 * slots - 2, (), 2 * slots - 2).wait()
            write(base, 2 * slots - 1, (pl.ds(0, write_head),), 2 * slots - 1).wait()

        wait_write_tail(units - slots)

    buf_bytes = slots * 16 * rows * W * x.dtype.itemsize
    out = pl.pallas_call(
        kernel,
        in_specs=[pl.BlockSpec(memory_space=pl.ANY)] * 3,
        out_specs=pl.BlockSpec(memory_space=pl.ANY),
        out_shape=jax.ShapeDtypeStruct((units, 16, rows, W), x.dtype),
        scratch_shapes=[
            pltpu.VMEM((slots, 16, rows, W), x.dtype),
            pltpu.VMEM((C,), g.dtype),
            pltpu.VMEM((C,), b.dtype),
            pltpu.VMEM((C, _LANES), jnp.float32),
            pltpu.VMEM((C, _LANES), jnp.float32),
            pltpu.SemaphoreType.DMA((slots + 1,)),
            pltpu.SemaphoreType.DMA((2 * slots + 1,)),
            pltpu.SemaphoreType.DMA((2,)),
        ],
        compiler_params=pltpu.CompilerParams(vmem_limit_bytes=buf_bytes + (6 << 20)),
    )(x.reshape(units, 16, rows, W), g, b)
    return out.reshape(x.shape)
```
